```python
import os as _os
_os.environ.setdefault("JAX_PLATFORMS", "cpu")
import jax
import jax.numpy as jnp

def _softmax(x, axis=-1):
    return jax.nn.softmax(x, axis=axis)
def _gelu(x):
    return jax.nn.gelu(x, approximate=True)
def _silu(x):
    return jax.nn.silu(x)
def _sigmoid(x):
    return jax.nn.sigmoid(x)
def _layernorm(x, axis=-1, eps=1e-5):
    m = jnp.mean(x, axis=axis, keepdims=True)
    v = jnp.var(x, axis=axis, keepdims=True)
    return (x - m) / jnp.sqrt(v + eps)
def _scatter_add(tgt, idx, src, axis=0):
    return tgt.at[idx].add(src)
def _segment_sum(src, seg, n):
    return jax.ops.segment_sum(src, seg, n)
class _Rng:
    def __init__(self, key):
        self._k = key
    def _next(self):
        self._k, sub = jax.random.split(self._k)
        return sub
    def normal(self, shape):
        return jax.random.normal(self._next(), shape, dtype=jnp.bfloat16)
    def randint(self, lo, hi, shape):
        return jax.random.randint(self._next(), shape, lo, hi, dtype=jnp.int32)
    def uniform(self, shape, lo=0.0, hi=1.0):
        return jax.random.uniform(self._next(), shape, jnp.bfloat16, lo, hi)
    def permutation(self, n):
        return jax.random.permutation(self._next(), n)


kernel_name = 'concat_heads__sliding_block_cached__sliding_block_cached__decode'

def setup_inputs():
    _rng = _Rng(jax.random.key(int.from_bytes(__import__("os").urandom(4), "little")))
    _w = (lambda a: (lambda t: t.astype(jnp.bfloat16) if jnp.issubdtype(t.dtype, jnp.floating) else t)(jnp.asarray(a)))
    def _A_setup():
        B, Sq, D = 1, 1, 640
        Hq, Hkv, Sk, Dh = 32, 32, 4096, 192
        assert Hq % Hkv == 0, (Hq, Hkv)
        return {
            "x": _w((lambda *s: _rng.normal(s) * 0.8)(B, Sq, D)),
            "k_cache": _w((lambda *s: _rng.normal(s) * 0.8)(B, Hkv, Sk, Dh)),
            "v_cache": _w((lambda *s: _rng.normal(s) * 0.05)(B, Hkv, Sk, Dh)),
            "wq": _w((lambda *s: _rng.normal(s) * 0.8)(D, Hq * Dh) * (D ** -0.5)),
            "wo": _w((lambda *s: _rng.normal(s) * 0.05)(Hq * Dh, D) * ((Hq * Dh) ** -0.5)),
        }
    _A_in = _A_setup()

    def _B_setup():
        B, Sq, D = 1, 1, 640
        Hq, Hkv, Sk, Dh = 32, 32, 4096, 192
        assert Hq % Hkv == 0, (Hq, Hkv)
        return {
            "x": _w((lambda *s: _rng.normal(s) * 0.8)(B, Sq, D)),
            "k_cache": _w((lambda *s: _rng.normal(s) * 0.8)(B, Hkv, Sk, Dh)),
            "v_cache": _w((lambda *s: _rng.normal(s) * 0.05)(B, Hkv, Sk, Dh)),
            "wq": _w((lambda *s: _rng.normal(s) * 0.8)(D, Hq * Dh) * (D ** -0.5)),
            "wo": _w((lambda *s: _rng.normal(s) * 0.05)(Hq * Dh, D) * ((Hq * Dh) ** -0.5)),
        }
    _B_in = _B_setup()

    return {
        "A_x": _A_in["x"],
        "A_k_cache": _A_in["k_cache"],
        "A_v_cache": _A_in["v_cache"],
        "A_wq": _A_in["wq"],
        "A_wo": _A_in["wo"],
        "B_x": _B_in["x"],
        "B_k_cache": _B_in["k_cache"],
        "B_v_cache": _B_in["v_cache"],
        "B_wq": _B_in["wq"],
        "B_wo": _B_in["wo"],
    }

def reference(A_x, A_k_cache, A_v_cache, A_wq, A_wo, B_x, B_k_cache, B_v_cache, B_wq, B_wo):
    def _A_ref(x, k_cache, v_cache, wq, wo):
        B, Sq, D = x.shape
        Hq, Dh = 32, 192
        Hkv, Sk = k_cache.shape[1], k_cache.shape[2]
        W = min(4096, max(256, Sk // 4))
        rep = Hq // Hkv
        q = (lambda x, *d: x.transpose(*d))((x @ wq).reshape(B, Sq, Hq, Dh), 0, 2, 1, 3)
        k = jnp.repeat(k_cache[:, :, Sk - W:, :], rep, axis=1)
        v = jnp.repeat(v_cache[:, :, Sk - W:, :], rep, axis=1)
        scores = jnp.einsum("bhqd,bhkd->bhqk", q, k) * (Dh ** -0.5)
        p = _softmax(scores, axis=-1)
        o = jnp.einsum("bhqk,bhkd->bhqd", p, v)
        return (lambda x, *d: x.transpose(*d))(o, 0, 2, 1, 3).reshape(B, Sq, Hq * Dh) @ wo

    def _B_ref(x, k_cache, v_cache, wq, wo):
        B, Sq, D = x.shape
        Hq, Dh = 32, 192
        Hkv, Sk = k_cache.shape[1], k_cache.shape[2]
        W = min(4096, max(256, Sk // 4))
        rep = Hq // Hkv
        q = (lambda x, *d: x.transpose(*d))((x @ wq).reshape(B, Sq, Hq, Dh), 0, 2, 1, 3)
        k = jnp.repeat(k_cache[:, :, Sk - W:, :], rep, axis=1)
        v = jnp.repeat(v_cache[:, :, Sk - W:, :], rep, axis=1)
        scores = jnp.einsum("bhqd,bhkd->bhqk", q, k) * (Dh ** -0.5)
        p = _softmax(scores, axis=-1)
        o = jnp.einsum("bhqk,bhkd->bhqd", p, v)
        return (lambda x, *d: x.transpose(*d))(o, 0, 2, 1, 3).reshape(B, Sq, Hq * Dh) @ wo

    a = _A_ref(A_x, A_k_cache, A_v_cache, A_wq, A_wo)
    b = _B_ref(B_x, B_k_cache, B_v_cache, B_wq, B_wo)
    return jnp.concatenate([a, b], axis=-1)
```

```python
import numpy as np
import jax
import jax.numpy as jnp
from jax import lax
import jax.experimental.pallas as pl
import jax.experimental.pallas.tpu as pltpu

H, DH, D = 32, 192, 640
G = 8
GR = G * DH
NG = H // G
TAIL = (1536, 1536, 1536, 1152, 256, 128)


def _kernel(ax, ak, av, awq, awo, bx, bk, bv, bwq, bwo, out,
            xb, qb, kb, vb, ob, qd, pd, ld, od, ov, sems):
    sk = ak.shape[1]
    w = kb.shape[1]
    n = [0]

    def start(src, dst):
        c = pltpu.make_async_copy(src, dst, sems.at[n[0]])
        n[0] += 1
        c.start()
        return c

    win = pl.ds(sk - w, w)
    cq = [start(awq, qb.at[0])]
    cx = [start(ax, xb.at[0]), start(bx, xb.at[1])]
    cq.append(start(bwq, qb.at[1]))
    ck = [start(ak.at[:, win], kb.at[pl.ds(0, H * DH)]),
          start(bk.at[:, win], kb.at[pl.ds(H * DH, H * DH)])]
    cv = [start(av.at[:, win], vb.at[pl.ds(0, H * DH)]),
          start(bv.at[:, win], vb.at[pl.ds(H * DH, H * DH)])]
    co = start(awo, ob.at[pl.ds(0, H * DH)])
    r = 0
    ct = []
    for t in TAIL:
        ct.append((r, t, start(bwo.at[pl.ds(r, t)], ob.at[pl.ds(H * DH + r, t)])))
        r += t

    row = lax.broadcasted_iota(jnp.int32, (G, GR), 0)
    col = lax.broadcasted_iota(jnp.int32, (G, GR), 1)
    diag = (col >= row * DH) & (col < (row + 1) * DH)

    def q_body(i, _):
        br = i // NG
        g = i % NG
        for b in range(2):
            @pl.when(i == b * NG)
            def _():
                cx[b].wait()
                cq[b].wait()
        x8 = jnp.broadcast_to(xb[br, 0].astype(jnp.float32), (G, D)).astype(jnp.bfloat16)
        q = jnp.dot(x8, qb[br, :, pl.ds(pl.multiple_of(g * GR, 128), GR)],
                    preferred_element_type=jnp.float32)
        qd[i] = jnp.where(diag, q, 0.0)
    lax.fori_loop(0, 2 * NG, q_body, None)

    def k_body(i, _):
        for b in range(2):
            @pl.when(i == b * NG)
            def _():
                ck[b].wait()
        s = jnp.dot(qd[i].astype(jnp.bfloat16), kb[pl.ds(pl.multiple_of(i * GR, GR), GR), :],
                    preferred_element_type=jnp.float32)
        s = s * np.float32(DH ** -0.5)
        m = jnp.max(s, axis=-1, keepdims=True)
        p = jnp.exp(s - m)
        pd[i] = p
        ld[i] = jnp.broadcast_to(jnp.sum(p, axis=-1, keepdims=True), (G, 128))
    lax.fori_loop(0, 2 * NG, k_body, None)

    def v_body(i, _):
        for b in range(2):
            @pl.when(i == b * NG)
            def _():
                cv[b].wait()
        o = lax.dot_general(pd[i].astype(jnp.bfloat16),
                            vb[pl.ds(pl.multiple_of(i * GR, GR), GR), :],
                            (((1,), (1,)), ((), ())), preferred_element_type=jnp.float32)
        o = o / ld[i][:, :1]
        od[i] = jnp.where(diag, o, 0.0)
    lax.fori_loop(0, 2 * NG, v_body, None)

    co.wait()

    def o_body(i, acc):
        return acc + jnp.dot(od[i].astype(jnp.bfloat16),
                             ob[pl.ds(pl.multiple_of(i * GR, GR), GR), :],
                             preferred_element_type=jnp.float32)
    acc = lax.fori_loop(0, NG, o_body, jnp.zeros((G, D), jnp.float32))
    ov[0, :, pl.ds(0, D)] = jnp.sum(acc, axis=0, keepdims=True).astype(ov.dtype)
    acc = jnp.zeros((G, D), jnp.float32)
    for r, t, c in ct:
        g, off = divmod(r, GR)
        lhs = od[NG + g, :, pl.ds(off, t)].astype(jnp.bfloat16)
        c.wait()
        acc = acc + jnp.dot(lhs, ob[pl.ds(H * DH + r, t), :], preferred_element_type=jnp.float32)
    ov[0, :, pl.ds(D, D)] = jnp.sum(acc, axis=0, keepdims=True).astype(ov.dtype)
    start(ov, out).wait()


@jax.jit
def pallas_concat_heads__sliding_block_cached__sliding_block_cached__decode_kernel(
    A_x: jax.Array,
    A_k_cache: jax.Array,
    A_v_cache: jax.Array,
    A_wq: jax.Array,
    A_wo: jax.Array,
    B_x: jax.Array,
    B_k_cache: jax.Array,
    B_v_cache: jax.Array,
    B_wq: jax.Array,
    B_wo: jax.Array,
):
    sk = A_k_cache.shape[2]
    w = min(4096, max(256, sk // 4))
    bf = jnp.bfloat16
    t = lambda a: jnp.swapaxes(a, 2, 3).reshape(H * DH, sk)
    return pl.pallas_call(
        _kernel,
        in_specs=[pl.BlockSpec(memory_space=pl.ANY)] * 10,
        out_specs=pl.BlockSpec(memory_space=pl.ANY),
        out_shape=jax.ShapeDtypeStruct((1, 1, 2 * D), bf),
        scratch_shapes=[
            pltpu.VMEM((2, 1, 1, D), bf),
            pltpu.VMEM((2, D, H * DH), bf),
            pltpu.VMEM((2 * H * DH, w), bf),
            pltpu.VMEM((2 * H * DH, w), bf),
            pltpu.VMEM((2 * H * DH, D), bf),
            pltpu.VMEM((2 * NG, G, GR), jnp.float32),
            pltpu.VMEM((2 * NG, G, w), jnp.float32),
            pltpu.VMEM((2 * NG, G, 128), jnp.float32),
            pltpu.VMEM((2 * NG, G, GR), jnp.float32),
            pltpu.VMEM((1, 1, 2 * D), bf),
            pltpu.SemaphoreType.DMA((10 + len(TAIL),)),
        ],
        compiler_params=pltpu.CompilerParams(
            vmem_limit_bytes=100 * 1024 * 1024,
            disable_semaphore_checks=True,
            disable_bounds_checks=True,
        ),
    )(A_x, t(A_k_cache), t(A_v_cache), A_wq, A_wo, B_x, t(B_k_cache), t(B_v_cache), B_wq, B_wo)
```

```python
import contextlib
import numpy as np
import jax, jax.numpy as jnp
from jax import lax
import jax.experimental.pallas as pl
import jax.experimental.pallas.tpu as pltpu

H, DH, SK, W, D = 32, 192, 4096, 1024, 640
N = H * DH
G = 8
GB = G * DH // 128
NB = N // 128
WS = [(2 * k) % 15 for k in range(15)]

def make(scope=False, compute=True, lag=2, tail=(8, 4, 2, 1), osplit=(8, 3, 2, 1, 1), settle=5, flags=None, kper=4, wper=5):
    sc = (lambda n: jax.named_scope(n)) if scope else (lambda n: contextlib.nullcontext())
    assert sum(tail) == 15 and sum(osplit) == 15
    def kern(ax, ak, av, awq, awo, bx, bk, bv, bwq, bwo, out, xb, qb, kb, vb, ob, qd, sd, pd, ld, od, md, ad, ov, sems):
        SX, SQ, SK_, SV, SOA, SOUT, SOB = 0, 1, 3, 5, 7, 8, 10
        ST = SOB + len(osplit)
        al = lambda v, m: v if isinstance(v, int) else pl.multiple_of(v, m)
        def dma(d, prio):
            pltpu.make_async_copy(d[0], d[1], sems.at[d[2]]).start(priority=prio)
        def wait(dst, sem):
            pltpu.make_async_copy(dst, dst, sems.at[sem]).wait()

        def round_q(br):
            def f(i):
                src = (awq, bwq)[br]
                rc = {}
                for b in (0, 2, 4):
                    a = ((i + b) * 43) >> 8
                    rc[b] = (a, i + b - 6 * a)
                res = []
                for s in WS:
                    a0, b = divmod(32 * s, 6)
                    idx = (pl.ds(al((rc[b][0] + a0) * 8, 8), 8), pl.ds(al(rc[b][1] * 1024, 1024), 1024))
                    res.append((src.at[idx], qb.at[(br,) + idx], SQ + br))
                return res
            return f, 32, wper
        def round_kv(src, dst, sem, br):
            def f(i):
                l = (i * 43) >> 8
                t = i - 6 * l
                r = al(((t & 1) * 8 + l) * 8, 8)
                j0 = (t >> 1) * 16
                return [(src.at[j0 + s, pl.ds(r, 8), pl.ds(SK - W, W)], dst.at[br * NB + j0 + s, pl.ds(r, 8)], sem + br) for s in range(16)]
            return f, 48, kper
        def round_o(br):
            def f(i):
                src = (awo, bwo)[br]
                if br == 0: sem = SOA
                else:
                    sem = SOB; e = 0
                    for n in osplit[:-1]:
                        e += 2 * n
                        sem = sem + (int(i >= e) if isinstance(i, int) else (i >= e).astype(jnp.int32))
                r = al(i * 64, 64)
                return [(src.at[s, pl.ds(r, 64)], ob.at[br, s, pl.ds(r, 64)], sem) for s in WS]
            return f, (32 if br == 0 else 30), wper
        last = []
        g = 0
        tgroups = []
        for gi, n in enumerate(tail):
            tgroups.append(WS[g:g + n]); g += n
            for u in (30, 31):
                for s in tgroups[-1]:
                    last.append((bwo.at[s, pl.ds(u * 64, 64)], ob.at[1, s, pl.ds(u * 64, 64)], ST + gi))

        def split(r, per):
            return [d for k, d in enumerate(r) if k % per != per - 1], [d for k, d in enumerate(r) if k % per == per - 1]
        def emit(slow, fast):
            n = len(slow) // len(fast) if fast else 0
            for k, d in enumerate(slow):
                dma(d, 1)
                if fast and k % n == n - 1: dma(fast[k // n], 0)

        row = lax.broadcasted_iota(jnp.int32, (G, 128), 0)
        col = lax.broadcasted_iota(jnp.int32, (G, 128), 1)
        def grp(j): return (j * 43) >> 9
        def diag(j):
            c = col + (j - grp(j) * GB) * 128 - row * DH
            return (c >= 0) & (c < DH)
        def q_step(br, i):
            x8 = jnp.broadcast_to(xb[br, 0].astype(jnp.float32), (G, D)).astype(jnp.bfloat16)
            q = jnp.dot(x8, qb[br, :, pl.ds(al(i * 256, 256), 256)], preferred_element_type=jnp.float32)
            for u in range(2):
                qd[br * NB + 2 * i + u] = jnp.where(diag(2 * i + u), q[:, u * 128:(u + 1) * 128], 0.0)
        def k_step(br, i):
            jj = br * NB + 2 * i
            q = jnp.concatenate([qd[jj], qd[jj + 1]], axis=1).astype(jnp.bfloat16)
            s = jnp.dot(q, kb[pl.ds(jj, 2)].reshape(256, W), preferred_element_type=jnp.float32)
            sd[grp(jj)] = sd[grp(jj)] + s
        def sm_step(g):
            s = sd[g] * np.float32(DH ** -0.5)
            p = jnp.exp(s - jnp.max(s, axis=-1, keepdims=True))
            pd[g] = p
            ld[g] = jnp.broadcast_to(1.0 / jnp.sum(p, axis=-1, keepdims=True), (G, 128))
        def v_step(br, i):
            jj = br * NB + 2 * i
            o = lax.dot_general(pd[grp(jj)].astype(jnp.bfloat16), vb[pl.ds(jj, 2)].reshape(256, W), (((1,), (1,)), ((), ())), preferred_element_type=jnp.float32)
            for u in range(2):
                od[pl.ds(jj + u, 1), :] = jnp.sum(jnp.where(diag(2 * i + u), o[:, u * 128:(u + 1) * 128] * ld[grp(jj)], 0.0), axis=0, keepdims=True)
        def expand(br):
            ei = lax.broadcasted_iota(jnp.int32, (128, 128), 0)
            ec = lax.broadcasted_iota(jnp.int32, (128, 128), 1)
            def body(u, _):
                o = od[pl.ds(br * NB, NB), :].astype(jnp.bfloat16)
                t = (ec >> 3) + 16 * u
                e = ((((t * 205) >> 10) * 8 + (ec & 7)) == ei).astype(jnp.float32).astype(jnp.bfloat16)
                md[br, u] = jnp.dot(o, e, preferred_element_type=jnp.float32)
            lax.fori_loop(0, 5, body, None)
        def lhs(br, t):
            j = (t * 205) >> 10
            u = t - 5 * j
            c = (col >> 3) + 16 * u
            keep = (c - 5 * ((c * 205) >> 10)) == row
            return jnp.where(keep, jnp.broadcast_to(md[br, u, pl.ds(j, 1), :], (G, 128)), 0.0).astype(jnp.bfloat16)
        def o_tiles(br, ss, u):
            l = jnp.concatenate([lhs(br, s * 16 + u) for s in ss], axis=1)
            return l, lambda: jnp.concatenate([ob[br, s, pl.ds(al(u * 128, 128), 128), :] for s in ss], axis=0)
        def o_step(i):
            br = i >> 4
            l, w = o_tiles(br, range(15), i & 15)
            ad[br] = ad[br] + jnp.dot(l, w(), preferred_element_type=jnp.float32)

        prev = [None]
        def phase(name, rnd, jobs=()):
            f, n, per = rnd
            with sc(name):
                def head(i, _):
                    fast = []
                    if prev[0] is not None:
                        pf, pn, pper = prev[0]
                        fast = split(pf(i + (pn - lag)), pper)[1]
                    emit(split(f(i), per)[0], fast)
                lax.fori_loop(0, lag, head, None)
                def body(i, _):
                    emit(split(f(i + lag), per)[0], split(f(i), per)[1])
                    for (a, m, fn_) in jobs:
                        assert a + m <= n - lag
                        @pl.when((i >= a) & (i < a + m))
                        def _(): fn_(i - a)
                lax.fori_loop(0, n - lag, body, None)
            prev[0] = rnd
        cj = lambda f: f if compute else (lambda j: None)
        s0 = settle

        phase("qa", round_q(0), [(0, 1, lambda j: (dma((ax, xb.at[0], SX), 0), dma((bx, xb.at[1], SX), 0))),
                                 (0, 8, lambda j: sd.__setitem__(j, jnp.zeros((G, W), jnp.float32)))])
        ad[...] = jnp.zeros(ad.shape, ad.dtype)
        phase("qb", round_q(1), [(s0, 1, lambda j: (wait(xb, SX), wait(qb.at[0], SQ))), (s0, 24, cj(lambda j: q_step(0, j)))])
        phase("ka", round_kv(ak, kb, SK_, 0), [(s0, 1, lambda j: wait(qb.at[1], SQ + 1)), (s0, 24, cj(lambda j: q_step(1, j)))])
        phase("kb", round_kv(bk, kb, SK_, 1), [(s0, 1, lambda j: wait(kb.at[pl.ds(0, NB)], SK_)), (s0, 24, cj(lambda j: k_step(0, j))), (s0 + 24, 4, cj(sm_step))])
        phase("va", round_kv(av, vb, SV, 0), [(s0, 1, lambda j: wait(kb.at[pl.ds(NB, NB)], SK_ + 1)), (s0, 24, cj(lambda j: k_step(1, j))), (s0 + 24, 4, cj(lambda j: sm_step(4 + j)))])
        phase("vb", round_kv(bv, vb, SV, 1), [(s0, 1, lambda j: wait(vb.at[pl.ds(0, NB)], SV)), (s0, 24, cj(lambda j: v_step(0, j))), (s0 + 24, 1, cj(lambda j: expand(0)))])
        phase("oa", round_o(0), [(s0, 1, lambda j: wait(vb.at[pl.ds(NB, NB)], SV + 1)), (s0, 24, cj(lambda j: v_step(1, j)))])
        n0 = 28 - s0
        assert n0 - 16 <= osplit[0]
        phase("ob", round_o(1), [(0, 1, cj(lambda j: expand(1))), (s0, 1, lambda j: wait(ob.at[0], SOA)),
                                 (s0 + 16, 1, lambda j: wait(ob.at[1, :, pl.ds(0, osplit[0] * 128)], SOB)), (s0, n0, cj(o_step))])
        with sc("ot"):
            f, n, per = prev[0]
            fast = sum([split(f(n - lag + i), per)[1] for i in range(lag)], [])
            emit(last[:24], fast); emit(last[24:], [])
        def put(br, acc):
            for j in range(5):
                ov[0, :, pl.ds(br * D + j * 128, 128)] = acc[j:j + 1].astype(ov.dtype)
        with sc("fin_b"):
            put(0, ad[0])
            def fin(i, _):
                e = osplit[0]
                for gi, n in enumerate(osplit[1:]):
                    @pl.when(i == 16 + e)
                    def _(): wait(ob.at[1, :, pl.ds(e * 128, n * 128)], SOB + 1 + gi)
                    e += n
                if compute: o_step(i)
            lax.fori_loop(n0, 31, fin, None)
        acc = ad[1]
        ls = [o_tiles(1, ss, 15) for ss in tgroups] if compute else None
        for gi, ss in enumerate(tgroups):
            with sc(f"fin_t{gi}"):
                wait(ob.at[1, pl.ds(0, len(ss)), pl.ds(15 * 128, 128)], ST + gi)
                if compute: acc = acc + jnp.dot(ls[gi][0], ls[gi][1](), preferred_element_type=jnp.float32)
        put(1, acc)
        c = pltpu.make_async_copy(ov, out, sems.at[SOUT]); c.start(); c.wait()

    def fn(ax, ak, av, awq, awo, bx, bk, bv, bwq, bwo):
        t = lambda a: jnp.swapaxes(a, 2, 3).reshape(NB, 128, SK)
        wo = lambda a: a.reshape(N // 8, 8, 5, 128).transpose(0, 2, 1, 3).reshape(15, 2048, 128)
        bf = jnp.bfloat16
        return pl.pallas_call(
            kern,
            in_specs=[pl.BlockSpec(memory_space=pl.ANY)] * 10,
            out_specs=pl.BlockSpec(memory_space=pl.ANY),
            out_shape=jax.ShapeDtypeStruct((1, 1, 2 * D), bf),
            scratch_shapes=[
                pltpu.VMEM((2, 1, 1, D), bf),
                pltpu.VMEM((2, D, N), bf),
                pltpu.VMEM((2 * NB, 128, W), bf),
                pltpu.VMEM((2 * NB, 128, W), bf),
                pltpu.VMEM((2, 15, 2048, 128), bf),
                pltpu.VMEM((2 * NB, G, 128), jnp.float32),
                pltpu.VMEM((8, G, W), jnp.float32),
                pltpu.VMEM((8, G, W), jnp.float32),
                pltpu.VMEM((8, G, 128), jnp.float32),
                pltpu.VMEM((2 * NB, 128), jnp.float32),
                pltpu.VMEM((2, 5, NB, 128), jnp.float32),
                pltpu.VMEM((2, G, 128), jnp.float32),
                pltpu.VMEM((1, 1, 2 * D), bf),
                pltpu.SemaphoreType.DMA((32,)),
            ],
            compiler_params=pltpu.CompilerParams(vmem_limit_bytes=100 * 1024 * 1024, disable_semaphore_checks=True, disable_bounds_checks=True, flags=flags),
        )(ax, t(ak), t(av), awq, wo(awo), bx, t(bk), t(bv), bwq, wo(bwo))
    return fn


@jax.jit
def pallas_concat_heads__sliding_block_cached__sliding_block_cached__decode_kernel(
    A_x, A_k_cache, A_v_cache, A_wq, A_wo, B_x, B_k_cache, B_v_cache, B_wq, B_wo,
):
    return make(tail=(11,4))(A_x, A_k_cache, A_v_cache, A_wq, A_wo, B_x, B_k_cache, B_v_cache, B_wq, B_wo)
```

```python
import numpy as np
import jax
import jax.numpy as jnp
from jax import lax
import jax.experimental.pallas as pl
import jax.experimental.pallas.tpu as pltpu

H, DH, D = 32, 192, 640
SK, W = 4096, 1024
N = H * DH
G = 8
NB = N // 128
GB = G * DH // 128
DB = D // 128

SWEEPS = 8
PERIOD, LAG = 4, 36
SEGS = [(2 * k) % 15 for k in range(15)]
W_ORDER = [(k, u) for u in range(4) for k in range(15)]
KV_ORDER = [(12 * b + s, h) for b in range(4) for h in range(2) for s in range(12)]
TAIL = (8, 4, 2, 1)

(SEM_X, SEM_QA, SEM_QB, SEM_KA, SEM_KB, SEM_VA, SEM_VB, SEM_OA, SEM_OUT, SEM_OB) = range(10)
SEM_TAIL = SEM_OB + SWEEPS

BF16, F32 = jnp.bfloat16, jnp.float32


def _div(v, d):
    return (v * -(-(1 << 16) // d)) >> 16


def _ds(start, size):
    if not isinstance(start, int):
        start = pl.multiple_of(start, size)
    return pl.ds(start, size)


def _dot(a, b, contract=0):
    return lax.dot_general(a.astype(BF16), b, (((1,), (contract,)), ((), ())),
                           preferred_element_type=F32)


def _kernel(ax, ak, av, awq, awo, bx, bk, bv, bwq, bwo, out,
            x_buf, wq_a, wq_b, k_a, k_b, v_a, v_b, wo_a, wo_b,
            q_buf, s_buf, p_buf, r_buf, o_buf, e_buf, acc_buf, c_buf, out_buf, sems):
    def start(copy, queue):
        src, dst, sem = copy
        pltpu.make_async_copy(src, dst, sems.at[sem]).start(priority=queue)

    def wait(filled, sem):
        pltpu.make_async_copy(filled, filled, sems.at[sem]).wait()

    def wq_piece(src, dst, sem):
        def piece(i, n):
            k, u = W_ORDER[n]
            m = 32 * SEGS[k] + u + 4 * i
            a = _div(m, 6)
            idx = (_ds(a * 8, 8), _ds((m - 6 * a) * 1024, 1024))
            return src.at[idx], dst.at[idx], sem
        return piece, len(W_ORDER)

    def kv_piece(src, dst, sem):
        def piece(i, n):
            j, h = KV_ORDER[n]
            rows = _ds(h * 64 + i * 8, 8)
            return src.at[j, rows, pl.ds(SK - W, W)], dst.at[j, rows], sem
        return piece, len(KV_ORDER)

    def wo_piece(src, dst, sem, order=W_ORDER):
        def piece(i, n):
            k, u = order[n]
            rows = _ds(i * 256 + u * 64, 64)
            return src.at[SEGS[k], rows], dst.at[k, rows], sem(i, k, u)
        return piece, len(order)

    row = lax.broadcasted_iota(jnp.int32, (G, 128), 0)
    col = lax.broadcasted_iota(jnp.int32, (G, 128), 1)

    def own_head(j):
        c = col + (j - _div(j, GB) * GB) * 128 - row * DH
        return (c >= 0) & (c < DH)

    def q_step(b, wq):
        def step(i):
            x = jnp.broadcast_to(x_buf[b, 0].astype(F32), (G, D))
            q = _dot(x, wq[:, _ds(i * 512, 512)])
            for u in range(4):
                j = 4 * i + u
                q_buf[b, j] = jnp.where(own_head(j), q[:, u * 128:(u + 1) * 128], 0.0)
        return step

    def k_step(b, k):
        def step(i):
            q = jnp.concatenate([q_buf[b, 4 * i + u] for u in range(4)], axis=1)
            g = _div(i, GB // 4)
            s_buf[b, g] += _dot(q, k[pl.ds(4 * i, 4)].reshape(512, W))
        return step

    def softmax(b):
        s = s_buf[b] * np.float32(DH ** -0.5)
        p = jnp.exp(s - jnp.max(s, axis=-1, keepdims=True))
        p_buf[b] = p
        r_buf[b] = jnp.broadcast_to(1.0 / jnp.sum(p, axis=-1, keepdims=True), (H // G, G, 128))

    def v_step(b, v):
        def step(i):
            g = _div(i, GB // 4)
            o = _dot(p_buf[b, g], v[pl.ds(4 * i, 4)].reshape(512, W), contract=1)
            for u in range(4):
                j = 4 * i + u
                o_j = jnp.where(own_head(j), o[:, u * 128:(u + 1) * 128] * r_buf[b, g], 0.0)
                o_buf[b, pl.ds(j, 1), :] = jnp.sum(o_j, axis=0, keepdims=True)
        return step

    def spread(b):
        src = lax.broadcasted_iota(jnp.int32, (128, D), 0)
        dst = lax.broadcasted_iota(jnp.int32, (128, D), 1)
        pick = _div(dst >> 3, DB) * 8 + (dst & 7) == src
        e = _dot(o_buf[b], pick.astype(F32).astype(BF16))
        for u in range(DB):
            e_buf[b, u] = e[:, u * 128:(u + 1) * 128]

    def wo_lhs(b, tiles):
        parts = []
        for k, t in tiles:
            j = _div(16 * SEGS[k] + t, DB)
            u = 16 * SEGS[k] + t - DB * j
            c = (col >> 3) + 16 * u
            e = jnp.broadcast_to(e_buf[b, u, pl.ds(j, 1), :], (G, 128))
            parts.append(jnp.where(c - DB * _div(c, DB) == row, e, 0.0).astype(BF16))
        return jnp.concatenate(parts, axis=1)

    def wo_rhs(wo, tiles):
        return jnp.concatenate([wo[k, _ds(t * 128, 128), :] for k, t in tiles], axis=0)

    def o_step(b, wo, t0, count):
        tiles = [(k, t0 + t) for t in range(count) for k in range(15)]
        acc_buf[b] += _dot(wo_lhs(b, tiles), wo_rhs(wo, tiles))

    def ob_sweep_step(i):
        wait(wo_b.at[:, _ds(i * 256, 256)], SEM_OB + i)
        o_step(1, wo_b, 2 * i, 2)

    def stream(array, before, first=None, ready=None, step=None, sweeps=SWEEPS):
        piece, size = array

        def issue(i, slots, late):
            for n in slots:
                if n % PERIOD != PERIOD - 1:
                    start(piece(i, n), 1)
                elif n >= LAG:
                    start(piece(i, n - LAG), 0)
                elif late is not None:
                    start(late(n - LAG), 0)

        issue(0, range(size), before and (lambda n: before[0](SWEEPS - 1, before[1] + n)))
        if first is not None:
            first()

        def sweep(i, _):
            for half in range(2):
                issue(i, range(half * size // 2, (half + 1) * size // 2),
                      lambda n: piece(i - 1, size + n))
                if ready is not None and half == 0:
                    pl.when(i == 2)(ready)
                if step is not None:
                    pl.when(i >= 2)(lambda: step(2 * (i - 2) + half))

        lax.fori_loop(1, sweeps, sweep, None)
        return array

    def setup():
        start((ax, x_buf.at[0], SEM_X), 0)
        start((bx, x_buf.at[1], SEM_X), 0)
        s_buf[...] = jnp.zeros(s_buf.shape, F32)
        acc_buf[...] = jnp.zeros(acc_buf.shape, F32)

    def last_step(i):
        pl.when(i < 8)(lambda: o_step(0, wo_a, 2 * i, 2))
        pl.when(i >= 8)(lambda: ob_sweep_step(i - 8))

    a = stream(wq_piece(awq, wq_a, SEM_QA), None, ready=setup)
    a = stream(wq_piece(bwq, wq_b, SEM_QB), a, lambda: wait(x_buf, SEM_X),
               lambda: wait(wq_a, SEM_QA), q_step(0, wq_a))
    a = stream(kv_piece(ak, k_a, SEM_KA), a, None, lambda: wait(wq_b, SEM_QB), q_step(1, wq_b))
    a = stream(kv_piece(bk, k_b, SEM_KB), a, None, lambda: wait(k_a, SEM_KA), k_step(0, k_a))
    a = stream(kv_piece(av, v_a, SEM_VA), a, lambda: softmax(0),
               lambda: wait(k_b, SEM_KB), k_step(1, k_b))
    a = stream(kv_piece(bv, v_b, SEM_VB), a, lambda: softmax(1),
               lambda: wait(v_a, SEM_VA), v_step(0, v_a))
    a = stream(wo_piece(awo, wo_a, lambda i, k, u: SEM_OA), a, lambda: spread(0),
               lambda: wait(v_b, SEM_VB), v_step(1, v_b))
    a = stream(wo_piece(bwo, wo_b, lambda i, k, u: SEM_OB + i), a, lambda: spread(1),
               lambda: wait(wo_a, SEM_OA), last_step, sweeps=SWEEPS - 1)
    for c in range(DB):
        out_buf[0, :, pl.ds(c * 128, 128)] = acc_buf[0, pl.ds(c, 1), :].astype(BF16)

    group = [g for g, n in enumerate(TAIL) for _ in range(n)]
    order = W_ORDER[:30] + [(k, u) for k in range(15) for u in (2, 3)]
    piece, size = wo_piece(
        bwo, wo_b, lambda i, k, u: SEM_OB + i if u < 2 else SEM_TAIL + group[k], order)
    plain = size - (LAG - LAG // PERIOD)
    slow = [n for n in range(size) if n % PERIOD != PERIOD - 1 or n >= plain]
    fast = list(range(PERIOD - 1 - LAG, plain, PERIOD))
    for m, n in enumerate(slow):
        start(piece(SWEEPS - 1, n), 1)
        if m % (PERIOD - 1) == PERIOD - 2 and fast:
            f = fast.pop(0)
            start(piece(SWEEPS - 1, f) if f >= 0 else a[0](SWEEPS - 2, size + f), 0)
        if m == 12:
            for k in range(TAIL[0], 15):
                j, u = divmod(16 * SEGS[k] + 15, DB)
                o_j = o_buf[1, pl.ds(j, 1), :].astype(BF16).astype(F32)
                lo = 16 * u // DB * 8
                c_buf[k - TAIL[0]] = jnp.broadcast_to(o_j, (128, 128)).T[lo:lo + 32]
        if m == 30:
            ob_sweep_step(2)
    assert not fast

    lax.fori_loop(3, SWEEPS - 1, lambda i, _: ob_sweep_step(i), None)
    wait(wo_b.at[:, pl.ds(14 * 128, 128)], SEM_OB + SWEEPS - 1)
    o_step(1, wo_b, 14, 1)

    tiles = [(k, 15) for k in range(TAIL[0])]
    lhs = wo_lhs(1, tiles)
    wait(wo_b.at[pl.ds(0, TAIL[0]), pl.ds(15 * 128, 128)], SEM_TAIL)
    acc = acc_buf[1] + _dot(lhs, wo_rhs(wo_b, tiles))
    acc = [jnp.where(row == c, acc, 0.0) for c in range(DB)]
    for g in range(1, len(TAIL)):
        k0 = sum(TAIL[:g])
        wait(wo_b.at[pl.ds(k0, TAIL[g]), pl.ds(15 * 128, 128)], SEM_TAIL + g)
        for k in range(k0, k0 + TAIL[g]):
            u = (16 * SEGS[k] + 15) % DB
            w = wo_b[k, pl.ds(15 * 128, 128), :].astype(F32)
            for t in range(16):
                r, c = divmod(16 * u + t, DB)
                o_r = c_buf[k - TAIL[0], pl.ds((r - 16 * u // DB) * 8, 8), :]
                acc[c] = acc[c] + w[8 * t:8 * t + 8] * o_r
    for c in range(DB):
        out_buf[0, :, pl.ds(D + c * 128, 128)] = jnp.sum(acc[c], axis=0, keepdims=True).astype(BF16)

    result = pltpu.make_async_copy(out_buf, out, sems.at[SEM_OUT])
    result.start()
    result.wait()


@jax.jit
def pallas_concat_heads__sliding_block_cached__sliding_block_cached__decode_kernel(
    A_x: jax.Array,
    A_k_cache: jax.Array,
    A_v_cache: jax.Array,
    A_wq: jax.Array,
    A_wo: jax.Array,
    B_x: jax.Array,
    B_k_cache: jax.Array,
    B_v_cache: jax.Array,
    B_wq: jax.Array,
    B_wo: jax.Array,
):
    def cache(a):
        return jnp.swapaxes(a, 2, 3).reshape(NB, 128, SK)

    def wo(a):
        return a.reshape(N // 8, 8, DB, 128).transpose(0, 2, 1, 3).reshape(15, 2048, 128)

    return pl.pallas_call(
        _kernel,
        in_specs=[pl.BlockSpec(memory_space=pl.ANY)] * 10,
        out_specs=pl.BlockSpec(memory_space=pl.ANY),
        out_shape=jax.ShapeDtypeStruct((1, 1, 2 * D), BF16),
        scratch_shapes=[
            pltpu.VMEM((2, 1, 1, D), BF16),
            *[pltpu.VMEM((D, N), BF16)] * 2,
            *[pltpu.VMEM((NB, 128, W), BF16)] * 4,
            *[pltpu.VMEM((15, 2048, 128), BF16)] * 2,
            pltpu.VMEM((2, NB, G, 128), F32),
            pltpu.VMEM((2, H // G, G, W), F32),
            pltpu.VMEM((2, H // G, G, W), F32),
            pltpu.VMEM((2, H // G, G, 128), F32),
            pltpu.VMEM((2, NB, 128), F32),
            pltpu.VMEM((2, DB, NB, 128), F32),
            pltpu.VMEM((2, G, 128), F32),
            pltpu.VMEM((15 - TAIL[0], 32, 128), F32),
            pltpu.VMEM((1, 1, 2 * D), BF16),
            pltpu.SemaphoreType.DMA((SEM_TAIL + len(TAIL),)),
        ],
        compiler_params=pltpu.CompilerParams(
            vmem_limit_bytes=100 * 1024 * 1024,
            disable_bounds_checks=True,
            disable_semaphore_checks=True,
        ),
    )(A_x, cache(A_k_cache), cache(A_v_cache), A_wq, wo(A_wo),
      B_x, cache(B_k_cache), cache(B_v_cache), B_wq, wo(B_wo))
```

```python
import numpy as np
import jax
import jax.numpy as jnp
from jax import lax
import jax.experimental.pallas as pl
import jax.experimental.pallas.tpu as pltpu

H, DH, D = 32, 192, 640
SK, W = 4096, 1024
N = H * DH
G = 8
NB = N // 128
GB = G * DH // 128
DB = D // 128

SWEEPS = 8
PERIOD, LAG = 4, 36
SEGS = [(2 * k) % 15 for k in range(15)]
W_ORDER = [(k, u) for u in range(4) for k in range(15)]
KV_ORDER = [(12 * b + s, h) for b in range(4) for h in range(2) for s in range(12)]
TAIL = (7, 5, 2, 1)

(SEM_X, SEM_QA, SEM_QB, SEM_KA, SEM_KB, SEM_VA, SEM_VB, SEM_OA, SEM_OUT, SEM_OB) = range(10)
SEM_TAIL = SEM_OB + SWEEPS

BF16, F32 = jnp.bfloat16, jnp.float32


def _div(v, d):
    return (v * -(-(1 << 16) // d)) >> 16


def _ds(start, size):
    if not isinstance(start, int):
        start = pl.multiple_of(start, size)
    return pl.ds(start, size)


def _dot(a, b, contract=0):
    return lax.dot_general(a.astype(BF16), b, (((1,), (contract,)), ((), ())),
                           preferred_element_type=F32)


def _kernel(ax, ak, av, awq, awo, bx, bk, bv, bwq, bwo, out,
            x_buf, wq_a, wq_b, k_a, k_b, v_a, v_b, wo_a, wo_b,
            q_buf, s_buf, p_buf, r_buf, o_buf, e_buf, acc_buf, c_buf, out_buf, sems):
    def start(copy, queue):
        src, dst, sem = copy
        pltpu.make_async_copy(src, dst, sems.at[sem]).start(priority=queue)

    def wait(filled, sem):
        pltpu.make_async_copy(filled, filled, sems.at[sem]).wait()

    def wq_piece(src, dst, sem):
        def piece(i, n):
            k, u = W_ORDER[n]
            m = 32 * SEGS[k] + u + 4 * i
            a = _div(m, 6)
            idx = (_ds(a * 8, 8), _ds((m - 6 * a) * 1024, 1024))
            return src.at[idx], dst.at[idx], sem
        return piece, len(W_ORDER)

    def kv_piece(src, dst, sem):
        def piece(i, n):
            j, h = KV_ORDER[n]
            rows = _ds(h * 64 + i * 8, 8)
            return src.at[j, rows, pl.ds(SK - W, W)], dst.at[j, rows], sem
        return piece, len(KV_ORDER)

    def wo_piece(src, dst, sem, order=W_ORDER):
        def piece(i, n):
            k, u = order[n]
            rows = _ds(i * 256 + u * 64, 64)
            return src.at[SEGS[k], rows], dst.at[k, rows], sem(i, k, u)
        return piece, len(order)

    row = lax.broadcasted_iota(jnp.int32, (G, 128), 0)
    col = lax.broadcasted_iota(jnp.int32, (G, 128), 1)

    def own_head(j):
        c = col + (j - _div(j, GB) * GB) * 128 - row * DH
        return (c >= 0) & (c < DH)

    def q_step(b, wq):
        def step(i):
            x = jnp.broadcast_to(x_buf[b, 0].astype(F32), (G, D))
            q = _dot(x, wq[:, _ds(i * 512, 512)])
            for u in range(4):
                j = 4 * i + u
                q_buf[b, j] = jnp.where(own_head(j), q[:, u * 128:(u + 1) * 128], 0.0)
        return step

    def k_step(b, k):
        def step(i):
            q = jnp.concatenate([q_buf[b, 4 * i + u] for u in range(4)], axis=1)
            g = _div(i, GB // 4)
            s_buf[b, g] += _dot(q, k[pl.ds(4 * i, 4)].reshape(512, W))
        return step

    def softmax(b):
        s = s_buf[b] * np.float32(DH ** -0.5)
        p = jnp.exp(s - jnp.max(s, axis=-1, keepdims=True))
        p_buf[b] = p
        r_buf[b] = jnp.broadcast_to(1.0 / jnp.sum(p, axis=-1, keepdims=True), (H // G, G, 128))

    def v_step(b, v):
        def step(i):
            g = _div(i, GB // 4)
            o = _dot(p_buf[b, g], v[pl.ds(4 * i, 4)].reshape(512, W), contract=1)
            for u in range(4):
                j = 4 * i + u
                o_j = jnp.where(own_head(j), o[:, u * 128:(u + 1) * 128] * r_buf[b, g], 0.0)
                o_buf[b, pl.ds(j, 1), :] = jnp.sum(o_j, axis=0, keepdims=True)
        return step

    def spread(b):
        src = lax.broadcasted_iota(jnp.int32, (128, D), 0)
        dst = lax.broadcasted_iota(jnp.int32, (128, D), 1)
        pick = _div(dst >> 3, DB) * 8 + (dst & 7) == src
        e = _dot(o_buf[b], pick.astype(F32).astype(BF16))
        for u in range(DB):
            c = (col >> 3) + 16 * u
            keep = c - DB * _div(c, DB) == row
            for j in range(NB):
                e_buf[b, DB * j + u] = jnp.where(keep, e[j:j + 1, u * 128:(u + 1) * 128], 0.0)

    def wo_lhs(b, tiles):
        return jnp.concatenate([e_buf[b, 16 * SEGS[k] + t] for k, t in tiles], axis=1)

    def wo_rhs(wo, tiles):
        return jnp.concatenate([wo[k, _ds(t * 128, 128), :] for k, t in tiles], axis=0)

    def o_step(b, wo, t0, count):
        tiles = [(k, t0 + t) for t in range(count) for k in range(15)]
        acc_buf[b] += _dot(wo_lhs(b, tiles), wo_rhs(wo, tiles))

    def ob_sweep_step(i):
        wait(wo_b.at[:, _ds(i * 256, 256)], SEM_OB + i)
        o_step(1, wo_b, 2 * i, 2)

    def stream(array, before, first=None, ready=None, step=None, sweeps=SWEEPS):
        piece, size = array

        def issue(i, slots, late):
            for n in slots:
                if n % PERIOD != PERIOD - 1:
                    start(piece(i, n), 1)
                elif n >= LAG:
                    start(piece(i, n - LAG), 0)
                elif late is not None:
                    start(late(n - LAG), 0)

        issue(0, range(size), before and (lambda n: before[0](SWEEPS - 1, before[1] + n)))
        if first is not None:
            first()

        def sweep(i, _):
            for half in range(2):
                issue(i, range(half * size // 2, (half + 1) * size // 2),
                      lambda n: piece(i - 1, size + n))
                if ready is not None and half == 0:
                    pl.when(i == 2)(ready)
                if step is not None:
                    pl.when(i >= 2)(lambda: step(2 * (i - 2) + half))

        lax.fori_loop(1, sweeps, sweep, None)
        return array

    def setup():
        start((ax, x_buf.at[0], SEM_X), 0)
        start((bx, x_buf.at[1], SEM_X), 0)
        s_buf[...] = jnp.zeros(s_buf.shape, F32)
        acc_buf[...] = jnp.zeros(acc_buf.shape, F32)

    def last_step(i):
        pl.when(i < 8)(lambda: o_step(0, wo_a, 2 * i, 2))
        pl.when(i >= 8)(lambda: ob_sweep_step(i - 8))

    a = stream(wq_piece(awq, wq_a, SEM_QA), None, ready=setup)
    a = stream(wq_piece(bwq, wq_b, SEM_QB), a, lambda: wait(x_buf, SEM_X),
               lambda: wait(wq_a, SEM_QA), q_step(0, wq_a))
    a = stream(kv_piece(ak, k_a, SEM_KA), a, None, lambda: wait(wq_b, SEM_QB), q_step(1, wq_b))
    a = stream(kv_piece(bk, k_b, SEM_KB), a, None, lambda: wait(k_a, SEM_KA), k_step(0, k_a))
    a = stream(kv_piece(av, v_a, SEM_VA), a, lambda: softmax(0),
               lambda: wait(k_b, SEM_KB), k_step(1, k_b))
    a = stream(kv_piece(bv, v_b, SEM_VB), a, lambda: softmax(1),
               lambda: wait(v_a, SEM_VA), v_step(0, v_a))
    a = stream(wo_piece(awo, wo_a, lambda i, k, u: SEM_OA), a, lambda: spread(0),
               lambda: wait(v_b, SEM_VB), v_step(1, v_b))
    a = stream(wo_piece(bwo, wo_b, lambda i, k, u: SEM_OB + i), a, lambda: spread(1),
               lambda: wait(wo_a, SEM_OA), last_step, sweeps=SWEEPS - 1)
    for c in range(DB):
        out_buf[0, :, pl.ds(c * 128, 128)] = acc_buf[0, pl.ds(c, 1), :].astype(BF16)

    group = [g for g, n in enumerate(TAIL) for _ in range(n)]
    order = W_ORDER[:30] + [(k, u) for k in range(15) for u in (2, 3)]
    piece, size = wo_piece(
        bwo, wo_b, lambda i, k, u: SEM_OB + i if u < 2 else SEM_TAIL + group[k], order)
    plain = size - (LAG - LAG // PERIOD)
    slow = [n for n in range(size) if n % PERIOD != PERIOD - 1 or n >= plain]
    fast = list(range(PERIOD - 1 - LAG, plain, PERIOD))
    for m, n in enumerate(slow):
        start(piece(SWEEPS - 1, n), 1)
        if m % (PERIOD - 1) == PERIOD - 2 and fast:
            f = fast.pop(0)
            start(piece(SWEEPS - 1, f) if f >= 0 else a[0](SWEEPS - 2, size + f), 0)
        if m == 12:
            for k in range(TAIL[0], 15):
                j, u = divmod(16 * SEGS[k] + 15, DB)
                o_j = o_buf[1, pl.ds(j, 1), :].astype(BF16).astype(F32)
                lo = 16 * u // DB * 8
                c_buf[k - TAIL[0]] = jnp.broadcast_to(o_j, (128, 128)).T[lo:lo + 32]
        if m == 30:
            ob_sweep_step(2)
    assert not fast

    lax.fori_loop(3, SWEEPS - 1, lambda i, _: ob_sweep_step(i), None)
    wait(wo_b.at[:, pl.ds(14 * 128, 128)], SEM_OB + SWEEPS - 1)
    o_step(1, wo_b, 14, 1)

    tiles = [(k, 15) for k in range(TAIL[0])]
    lhs = wo_lhs(1, tiles).astype(BF16)
    wait(wo_b.at[pl.ds(0, TAIL[0]), pl.ds(15 * 128, 128)], SEM_TAIL)
    acc = acc_buf[1] + _dot(lhs, wo_rhs(wo_b, tiles))
    acc = [jnp.where(row == c, acc, 0.0) for c in range(DB)]
    for g in range(1, len(TAIL)):
        k0 = sum(TAIL[:g])
        wait(wo_b.at[pl.ds(k0, TAIL[g]), pl.ds(15 * 128, 128)], SEM_TAIL + g)
        for k in range(k0, k0 + TAIL[g]):
            u = (16 * SEGS[k] + 15) % DB
            w = wo_b[k, pl.ds(15 * 128, 128), :].astype(F32)
            for t in range(16):
                r, c = divmod(16 * u + t, DB)
                o_r = c_buf[k - TAIL[0], pl.ds((r - 16 * u // DB) * 8, 8), :]
                acc[c] = acc[c] + w[8 * t:8 * t + 8] * o_r
    for c in range(DB):
        out_buf[0, :, pl.ds(D + c * 128, 128)] = jnp.sum(acc[c], axis=0, keepdims=True).astype(BF16)

    result = pltpu.make_async_copy(out_buf, out, sems.at[SEM_OUT])
    result.start()
    result.wait()


@jax.jit
def pallas_concat_heads__sliding_block_cached__sliding_block_cached__decode_kernel(
    A_x: jax.Array,
    A_k_cache: jax.Array,
    A_v_cache: jax.Array,
    A_wq: jax.Array,
    A_wo: jax.Array,
    B_x: jax.Array,
    B_k_cache: jax.Array,
    B_v_cache: jax.Array,
    B_wq: jax.Array,
    B_wo: jax.Array,
):
    def cache(a):
        return jnp.swapaxes(a, 2, 3).reshape(NB, 128, SK)

    def wo(a):
        return a.reshape(N // 8, 8, DB, 128).transpose(0, 2, 1, 3).reshape(15, 2048, 128)

    return pl.pallas_call(
        _kernel,
        in_specs=[pl.BlockSpec(memory_space=pl.ANY)] * 10,
        out_specs=pl.BlockSpec(memory_space=pl.ANY),
        out_shape=jax.ShapeDtypeStruct((1, 1, 2 * D), BF16),
        scratch_shapes=[
            pltpu.VMEM((2, 1, 1, D), BF16),
            *[pltpu.VMEM((D, N), BF16)] * 2,
            *[pltpu.VMEM((NB, 128, W), BF16)] * 4,
            *[pltpu.VMEM((15, 2048, 128), BF16)] * 2,
            pltpu.VMEM((2, NB, G, 128), F32),
            pltpu.VMEM((2, H // G, G, W), F32),
            pltpu.VMEM((2, H // G, G, W), F32),
            pltpu.VMEM((2, H // G, G, 128), F32),
            pltpu.VMEM((2, NB, 128), F32),
            pltpu.VMEM((2, NB * DB, G, 128), F32),
            pltpu.VMEM((2, G, 128), F32),
            pltpu.VMEM((15 - TAIL[0], 32, 128), F32),
            pltpu.VMEM((1, 1, 2 * D), BF16),
            pltpu.SemaphoreType.DMA((SEM_TAIL + len(TAIL),)),
        ],
        compiler_params=pltpu.CompilerParams(
            vmem_limit_bytes=100 * 1024 * 1024,
            disable_bounds_checks=True,
            disable_semaphore_checks=True,
        ),
    )(A_x, cache(A_k_cache), cache(A_v_cache), A_wq, wo(A_wo),
      B_x, cache(B_k_cache), cache(B_v_cache), B_wq, wo(B_wo))
```
